```python
import os as _os
_os.environ.setdefault("JAX_PLATFORMS", "cpu")
import jax
import jax.numpy as jnp

def _softmax(x, axis=-1):
    return jax.nn.softmax(x, axis=axis)
def _gelu(x):
    return jax.nn.gelu(x, approximate=True)
def _silu(x):
    return jax.nn.silu(x)
def _sigmoid(x):
    return jax.nn.sigmoid(x)
def _layernorm(x, axis=-1, eps=1e-5):
    m = jnp.mean(x, axis=axis, keepdims=True)
    v = jnp.var(x, axis=axis, keepdims=True)
    return (x - m) / jnp.sqrt(v + eps)
def _scatter_add(tgt, idx, src, axis=0):
    return tgt.at[idx].add(src)
def _segment_sum(src, seg, n):
    return jax.ops.segment_sum(src, seg, n)
class _Rng:
    def __init__(self, key):
        self._k = key
    def _next(self):
        self._k, sub = jax.random.split(self._k)
        return sub
    def normal(self, shape):
        return jax.random.normal(self._next(), shape, dtype=jnp.bfloat16)
    def randint(self, lo, hi, shape):
        return jax.random.randint(self._next(), shape, lo, hi, dtype=jnp.int32)
    def uniform(self, shape, lo=0.0, hi=1.0):
        return jax.random.uniform(self._next(), shape, jnp.bfloat16, lo, hi)
    def permutation(self, n):
        return jax.random.permutation(self._next(), n)


kernel_name = 'interleave_layers__linear_attn_block__mha_block__prompt'

def setup_inputs():
    _rng = _Rng(jax.random.key(int.from_bytes(__import__("os").urandom(4), "little")))
    _w = (lambda a: (lambda t: t.astype(jnp.bfloat16) if jnp.issubdtype(t.dtype, jnp.floating) else t)(jnp.asarray(a)))
    def _A_setup():
        B, S, D = 1, 2048, 1024
        return {
            "x": _w((lambda *s: _rng.normal(s) * 0.05)(B, S, D)),
            "wqkv": _w((lambda *s: _rng.normal(s) * 0.1)(D, 3 * D)),
            "wo": _w((lambda *s: _rng.normal(s) * 0.1)(D, D)),
        }
    _A_in = _A_setup()

    def _B_setup():
        B, S, D, H = 1, 2048, 1024, 32
        return {
            "x": _w((lambda *s: _rng.normal(s) * 0.05)(B, S, D)),
            "wqkv": _w((lambda *s: _rng.normal(s) * 0.1)(D, 3 * D)),
            "wo": _w((lambda *s: _rng.normal(s) * 0.05)(D, D)),
        }
    _B_in = _B_setup()

    return {
        "A_x": _A_in["x"],
        "A_wqkv": _A_in["wqkv"],
        "A_wo": _A_in["wo"],
        "B_x": _B_in["x"],
        "B_wqkv": _B_in["wqkv"],
        "B_wo": _B_in["wo"],
    }

def reference(A_x, A_wqkv, A_wo, B_x, B_wqkv, B_wo):
    def _A_ref(x, wqkv, wo):
        B, S, D = x.shape
        H = 32; Dh = D // H
        qkv = (lambda x, *d: x.transpose(*d))((x @ wqkv).reshape(B, S, 3, H, Dh), 2, 0, 3, 1, 4)
        q, k, v = qkv[0], qkv[1], qkv[2]
        phi = lambda t: jnp.where(t > 0, t + 1, jnp.exp(t)) + 1e-6
        pq, pk = phi(q), phi(k)
        kv = jnp.einsum("bhsd,bhse->bhde", pk, v)
        z = jnp.einsum("bhsd->bhd", pk)
        num = jnp.einsum("bhqd,bhde->bhqe", pq, kv)
        den = jnp.einsum("bhqd,bhd->bhq", pq, z)[..., None] + 1e-6
        o = num / den
        return (lambda x, *d: x.transpose(*d))(o, 0, 2, 1, 3).reshape(B, S, D) @ wo

    def _B_ref(x, wqkv, wo):
        B, S, D = x.shape
        H = 32
        Dh = D // H
        qkv = (lambda x, *d: x.transpose(*d))((x @ wqkv).reshape(B, S, 3, H, Dh), 2, 0, 3, 1, 4)
        q, k, v = qkv[0], qkv[1], qkv[2]
        scores = jnp.einsum("bhqd,bhkd->bhqk", q, k) * (Dh ** -0.5)
        p = _softmax(scores, axis=-1)
        o = jnp.einsum("bhqk,bhkd->bhqd", p, v)
        return (lambda x, *d: x.transpose(*d))(o, 0, 2, 1, 3).reshape(B, S, D) @ wo

    x = A_x
    x = x + _A_ref(_layernorm(x, axis=-1), A_wqkv, A_wo)
    x = x + _B_ref(_layernorm(x, axis=-1), B_wqkv, B_wo)
    x = x + _A_ref(_layernorm(x, axis=-1), A_wqkv, A_wo)
    x = x + _B_ref(_layernorm(x, axis=-1), B_wqkv, B_wo)
    return x
```

```python
import math

import jax
import jax.numpy as jnp
from jax import lax
import jax.experimental.pallas as pl
import jax.experimental.pallas.tpu as pltpu

S, D, H, DH = 2048, 1024, 32, 32
NG = D // 128
TM = 256
HM = 128
NT_ROWS = S // TM
TO = 512
HO = 256
TQ = 512
KC = 128
LAG = 3
U = 8
NQ = S // TQ
NKC = S // KC
NIT = H * NQ
QSCALE = (DH ** -0.5) * math.log2(math.e)
NT = (((1,), (1,)), ((), ()))
F32 = jnp.float32
BF16 = jnp.bfloat16


def _dot(a, b):
    return jnp.dot(a, b, preferred_element_type=F32)


def _dot_nt(a, b):
    return lax.dot_general(a, b, NT, preferred_element_type=F32)


def _phi(t):
    return jnp.where(t > 0, t + 1.0, jnp.exp(t)) + 1e-6


def _recip(d):
    r = pl.reciprocal(d, approx=True)
    return r * (2.0 - d * r)


def _ln(x):
    m = jnp.mean(x, axis=-1, keepdims=True)
    xc = x - m
    v = jnp.mean(xc * xc, axis=-1, keepdims=True)
    return (xc * lax.rsqrt(v + 1e-5)).astype(BF16)


def _cat(ref, b0, n, rows=None):
    if rows is None:
        return jnp.concatenate([ref[b0 + j] for j in range(n)], axis=1)
    return jnp.concatenate([ref[b0 + j, rows, :] for j in range(n)], axis=1)


def _kernel(x_hbm, wa_hbm, woa_hbm, wb_hbm, wob_hbm, out_hbm,
            xb, xres, wa, woa, wb, wob, q_s, k_s, vt_s,
            xna, xnb, kv_acc, zp, kz, m_ref, mp_ref, ot_buf, l_buf, zs, xsem, wsem, *sbufs):

    def x_copy(i):
        return pltpu.make_async_copy(x_hbm.at[pl.ds(i * TM, TM)], xb.at[pl.ds(i * TM, TM)], xsem.at[i])

    def out_copy(i):
        return pltpu.make_async_copy(xb.at[pl.ds(i * TO, TO)], out_hbm.at[pl.ds(i * TO, TO)], xsem.at[i])

    def w_group(src, dst, b0, sem):
        return [pltpu.make_async_copy(src.at[:, pl.ds((b0 + j) * 128, 128)], dst.at[b0 + j], wsem.at[sem])
                for j in range(NG)]

    g_wkv = w_group(wa_hbm, wa, NG, 0) + w_group(wa_hbm, wa, 2 * NG, 0)
    g_rest = (w_group(wa_hbm, wa, 0, 1) + w_group(woa_hbm, woa, 0, 1) + w_group(wb_hbm, wb, 2 * NG, 1)
              + w_group(wb_hbm, wb, 0, 1) + w_group(wb_hbm, wb, NG, 1) + w_group(wob_hbm, wob, 0, 1))
    x_copy(0).start()
    x_copy(0).wait()
    for c in g_wkv:
        c.start()
    x_copy(1).start()

    for i in range(8):
        zs[i] = 0

    def init_body(i, c):
        r0 = pl.multiple_of(i * 8, 8)
        for sb in sbufs:
            sb[:, pl.ds(r0, 8), :] = jnp.zeros((2, 8, TQ), F32)
        return c
    lax.fori_loop(0, KC // 8, init_body, 0)
    ot_buf[...] = jnp.zeros_like(ot_buf)
    l_buf[...] = jnp.ones_like(l_buf)

    def ln_tile(first, r0, dst, slot):
        rows = pl.ds(r0, HM)
        x = jnp.where(first, xb[rows, :].astype(F32), xres[rows, :])
        xres[rows, :] = x
        xn = _ln(x)
        for j in range(NG):
            dst[slot, j] = xn[:, j * 128:(j + 1) * 128]

    def ld_xn(src, slot):
        return jnp.concatenate([src[slot, j] for j in range(NG)], axis=1)

    def a_q(xn):
        return _phi(_dot(xn, _cat(wa, 0, NG))).astype(BF16)

    def a_k(xn):
        pk = _phi(_dot(xn, _cat(wa, NG, NG)))
        zrow = jnp.sum(pk.reshape(HM // 8, 8, D), axis=0)
        return pk.T.astype(BF16), zrow

    def a_v(xn):
        return _dot(xn, _cat(wa, 2 * NG, NG)).astype(BF16)

    def a_mid():
        r = lax.broadcasted_iota(jnp.int32, (128, 128), 0) // DH
        c = lax.broadcasted_iota(jnp.int32, (128, 128), 1) // DH
        bd = r == c
        for g in range(NG):
            z = jnp.sum(zp[:, g * 128:(g + 1) * 128], axis=0, keepdims=True)
            kz[2 * g] = jnp.where(bd, kv_acc[g], 0.0).astype(BF16)
            kz[2 * g + 1] = jnp.where(bd, jnp.broadcast_to(z, (128, 128)), 0.0).T.astype(BF16)

    def a_out(pq, r0):
        rows = pl.ds(r0, HM)
        os_ = []
        for g in range(NG):
            nd = _dot(pq[:, g * 128:(g + 1) * 128], _cat(kz, 2 * g, 2))
            os_.append((nd[:, 0:128] * _recip(nd[:, 128:256] + 1e-6)).astype(BF16))
        o = jnp.concatenate(os_, axis=1)
        x = xres[rows, :] + _dot(o, _cat(woa, 0, NG))
        xres[rows, :] = x
        return x

    def b_proj(xn, r0, blk):
        rows = pl.ds(r0, HM)
        vt_s[blk] = _dot(xn, _cat(wb, 2 * NG, NG)).T.astype(BF16)
        q = (_dot(xn, _cat(wb, 0, NG)) * QSCALE).astype(BF16)
        for g in range(NG):
            q_s[g, rows, :] = q[:, g * 128:(g + 1) * 128]
        k = _dot(xn, _cat(wb, NG, NG)).astype(BF16)
        for g in range(NG):
            k_s[g, rows, :] = k[:, g * 128:(g + 1) * 128]

    lane_head = lax.broadcasted_iota(jnp.int32, (TQ, 128), 1) // DH

    def tidx(t):
        gq = t // 4
        return gq // NQ, gq % NQ

    def get_q(t, j):
        g, qi = tidx(t)
        qg = q_s[g, pl.ds(pl.multiple_of(qi * TQ, TQ), TQ), :]
        return jnp.where(lane_head == j, qg.astype(F32), 0.0).astype(BF16)

    def qk_chunk(t, qm, c, slot, m):
        g, _ = tidx(t)
        s = _dot_nt(k_s[g, c * KC:(c + 1) * KC, :], qm)
        sbufs[c][slot] = s
        cm = jnp.max(s.reshape(KC // 8, 8, TQ), axis=0)
        return cm if m is None else jnp.maximum(m, cm)

    def pv_chunk(t, j, c, slot, mb, acc, l):
        g, _ = tidx(t)
        s = sbufs[c][slot]
        p = jnp.exp2(s.reshape(KC // 8, 8, TQ) - mb[None])
        a = None
        for r in range(7, -1, -1):
            pr = p[2 * r] + p[2 * r + 1]
            a = pr if a is None else a + pr
        pb = p.reshape(KC, TQ).astype(BF16)
        vt = vt_s[c, pl.ds(pl.multiple_of(g * 128 + j * DH, DH), DH), :]
        o = _dot(vt, pb)
        return (o if acc is None else acc + o), (a if l is None else l + a)

    def bcast_max(m):
        return jnp.broadcast_to(jnp.max(m, axis=0, keepdims=True), (8, TQ))

    def finalize(par, g, qi):
        parts = []
        for j in range(4):
            ls = jnp.sum(l_buf[par, j], axis=0, keepdims=True)
            parts.append(ot_buf[par, j * DH:(j + 1) * DH, :] * _recip(ls))
        ot = jnp.concatenate(parts, axis=0)
        q_s[g, pl.ds(pl.multiple_of(qi * TQ, TQ), TQ), :] = ot.T.astype(BF16)

    def attention():
        z0 = zs[0]
        qm = get_q(0, 0)
        m = None
        for c in range(NKC):
            m = qk_chunk(0, qm, c, z0, m)
        m_ref[...] = bcast_max(m)
        qm = get_q(1, 1)
        m = None
        for c in range(LAG):
            m = qk_chunk(1, qm, c, 1 - z0, m)
        mp_ref[...] = m

        def body(i, carry):
            t0 = i * U
            mb = m_ref[...]
            mp = mp_ref[...]
            qm1 = get_q(t0 + 1, 1)
            for u in range(U):
                t = t0 + u
                rs = (u + zs[(i + 2 * u) & 7]) & 1
                w1 = (u + 1 + zs[(i + 2 * u + 1) & 7]) & 1
                w2 = 1 - w1
                t1 = jnp.minimum(t + 1, NIT - 1)
                t2 = jnp.minimum(t + 2, NIT - 1)
                acc = None
                l = None
                m2 = None
                mb_next = None
                qm2 = None
                for c in range(NKC):
                    cq = c + LAG
                    if cq < NKC:
                        mp = qk_chunk(t1, qm1, cq, w1, mp)
                        if cq == NKC - 1:
                            mb_next = bcast_max(mp)
                    else:
                        if qm2 is None:
                            qm2 = get_q(t2, (u + 2) % 4)
                        m2 = qk_chunk(t2, qm2, cq - NKC, w2, m2)
                    acc, l = pv_chunk(t, u % 4, c, rs, mb, acc, l)
                if u % 4 == 0:
                    par = ((u // 4) + 1) % 2
                    g, qi = tidx(jnp.maximum(t - 1, 0))
                    if u == 0:
                        g = jnp.where(i == 0, NG, g)
                    finalize(par, g, qi)
                par = (u // 4) % 2
                ot_buf[par, (u % 4) * DH:(u % 4 + 1) * DH, :] = acc
                l_buf[par, u % 4] = l
                mb = mb_next
                mp = m2
                qm1 = qm2
            m_ref[...] = mb
            mp_ref[...] = mp
            return carry
        lax.fori_loop(0, NIT // U, body, 0)
        finalize((U // 4 - 1) % 2, NG - 1, NQ - 1)

    def pair(it, carry):
        first = it == 0

        kv_acc[...] = jnp.zeros_like(kv_acc)
        zp[...] = jnp.zeros_like(zp)

        z0 = zs[1]
        ln_tile(first, 0, xna, z0)
        ln_tile(first, HM, xnb, z0)

        @pl.when(first)
        def _():
            for c in g_wkv:
                c.wait()
            for i in range(2, NT_ROWS):
                x_copy(i).start()

        def loop_a(i, c):
            @pl.when(jnp.logical_and(first, i + 1 < NT_ROWS))
            def _():
                x_copy(i + 1).wait()

            @pl.when(jnp.logical_and(first, i == 1))
            def _():
                for c in g_rest:
                    c.start()

            cur = (i + zs[i & 7]) & (NT_ROWS - 1)
            inx = jnp.minimum(i + 1, NT_ROWS - 1)
            nxt = (inx + zs[(i + 1) & 7]) & (NT_ROWS - 1)
            rn = pl.multiple_of(inx * TM, TM)
            ln_tile(first, rn + HM, xnb, nxt)
            pka, za = a_k(ld_xn(xna, cur))
            ln_tile(first, rn, xna, nxt)
            pkb, zb = a_k(ld_xn(xnb, cur))
            zp[...] += za + zb
            pkt = jnp.concatenate([pka, pkb], axis=1)
            va = a_v(ld_xn(xna, cur))
            vb = a_v(ld_xn(xnb, cur))
            v = jnp.concatenate([va, vb], axis=0)
            for g in range(NG):
                kv_acc[g] += _dot(pkt[g * 128:(g + 1) * 128, :], v[:, g * 128:(g + 1) * 128])
            return c
        with jax.named_scope('loopA'):
            lax.fori_loop(0, NT_ROWS, loop_a, 0)

        @pl.when(first)
        def _():
            for c in g_rest:
                c.wait()

        a_mid()

        def loop2(i, c):
            pqs = [a_q(ld_xn(xna, i)), a_q(ld_xn(xnb, i))]
            xns = []
            for hh in range(TM // HM):
                r0 = pl.multiple_of(i * TM + hh * HM, HM)
                xns.append((_ln(a_out(pqs[hh], r0)), r0, i * (TM // HM) + hh))
            for xn, r0, blk in xns:
                b_proj(xn, r0, blk)
            return c
        with jax.named_scope('loop2'):
            lax.fori_loop(0, NT_ROWS, loop2, 0)

        with jax.named_scope('attn'):
            attention()

        def loop_o(i, c):
            for hh in range(TO // HO):
                rows = pl.ds(pl.multiple_of(i * TO + hh * HO, HO), HO)
                x = xres[rows, :] + _dot(_cat(q_s, 0, NG, rows), _cat(wob, 0, NG))
                xres[rows, :] = x
                xb[rows, :] = x.astype(BF16)

            @pl.when(it == 1)
            def _():
                out_copy(i).start()
            return c
        with jax.named_scope('loopO'):
            lax.fori_loop(0, S // TO, loop_o, 0)
        return carry
    lax.fori_loop(0, 2, pair, 0)

    for i in range(S // TO):
        out_copy(i).wait()


@jax.jit
def pallas_interleave_layers__linear_attn_block__mha_block__prompt_kernel(
    A_x: jax.Array,
    A_wqkv: jax.Array,
    A_wo: jax.Array,
    B_x: jax.Array,
    B_wqkv: jax.Array,
    B_wo: jax.Array,
):
    x = A_x.reshape(S, D)
    scratch = [
        pltpu.VMEM((S, D), BF16),
        pltpu.VMEM((S, D), F32),
        pltpu.VMEM((3 * NG, D, 128), BF16),
        pltpu.VMEM((NG, D, 128), BF16),
        pltpu.VMEM((3 * NG, D, 128), BF16),
        pltpu.VMEM((NG, D, 128), BF16),
        pltpu.VMEM((NG + 1, S, 128), BF16),
        pltpu.VMEM((NG, S, 128), BF16),
        pltpu.VMEM((NKC, D, 128), BF16),
        pltpu.VMEM((NT_ROWS, NG, HM, 128), BF16),
        pltpu.VMEM((NT_ROWS, NG, HM, 128), BF16),
        pltpu.VMEM((NG, 128, 128), F32),
        pltpu.VMEM((8, D), F32),
        pltpu.VMEM((2 * NG, 128, 128), BF16),
        pltpu.VMEM((8, TQ), F32),
        pltpu.VMEM((8, TQ), F32),
        pltpu.VMEM((2, 128, TQ), F32),
        pltpu.VMEM((2, 4, 8, TQ), F32),
        pltpu.SMEM((8,), jnp.int32),
        pltpu.SemaphoreType.DMA((NT_ROWS,)),
        pltpu.SemaphoreType.DMA((2,)),
    ] + [pltpu.VMEM((2, KC, TQ), F32) for _ in range(NKC)]
    out = pl.pallas_call(
        _kernel,
        out_shape=jax.ShapeDtypeStruct((S, D), BF16),
        in_specs=[pl.BlockSpec(memory_space=pl.ANY)] * 5,
        out_specs=pl.BlockSpec(memory_space=pl.ANY),
        scratch_shapes=scratch,
        compiler_params=pltpu.CompilerParams(vmem_limit_bytes=110 * 1024 * 1024),
    )(x, A_wqkv, A_wo, B_wqkv, B_wo)
    return out.reshape(1, S, D)
```

```python
import math

import jax
import jax.numpy as jnp
from jax import lax
import jax.experimental.pallas as pl
import jax.experimental.pallas.tpu as pltpu

S, D, H, DH = 2048, 1024, 32, 32
NG = D // 128
TM = 256
HM = 128
NT_ROWS = S // TM
PO = 256
TO = 448
HO = 224
NO = (S - PO) // TO
TQ = 512
KC = 128
LAG = 3
U = 8
NQ = S // TQ
NKC = S // KC
NIT = H * NQ
QSCALE = (DH ** -0.5) * math.log2(math.e)
NT = (((1,), (1,)), ((), ()))
F32 = jnp.float32
BF16 = jnp.bfloat16


def _dot(a, b):
    return jnp.dot(a, b, preferred_element_type=F32)


def _dot_nt(a, b):
    return lax.dot_general(a, b, NT, preferred_element_type=F32)


def _phi(t):
    return jnp.where(t > 0, t + 1.0, jnp.exp(t)) + 1e-6


def _recip(d):
    r = pl.reciprocal(d, approx=True)
    return r * (2.0 - d * r)


def _ln(x):
    m = jnp.mean(x, axis=-1, keepdims=True)
    xc = x - m
    v = jnp.mean(xc * xc, axis=-1, keepdims=True)
    return (xc * lax.rsqrt(v + 1e-5)).astype(BF16)


def _cat(ref, b0, n, rows=None):
    if rows is None:
        return jnp.concatenate([ref[b0 + j] for j in range(n)], axis=1)
    return jnp.concatenate([ref[b0 + j, rows, :] for j in range(n)], axis=1)


def _kernel(x_hbm, wa_hbm, woa_hbm, wb_hbm, wob_hbm, out_hbm,
            xb, xres, wa, woa, wb, wob, q_s, k_s, vt_s,
            xna, xnb, g_acc, zp, m_s, zsel, m_ref, acc_ref, lc_ref, ot_buf, l_buf, zs, xsem, wsem, *sbufs):

    def x_copy(i):
        return pltpu.make_async_copy(x_hbm.at[pl.ds(i * TM, TM)], xb.at[pl.ds(i * TM, TM)], xsem.at[i])

    def out_copy(r0, n, k):
        return pltpu.make_async_copy(xb.at[pl.ds(r0, n)], out_hbm.at[pl.ds(r0, n)], xsem.at[k])

    def w_group(src, dst, b0, sem):
        return [pltpu.make_async_copy(src.at[:, pl.ds((b0 + j) * 128, 128)], dst.at[b0 + j], wsem.at[sem])
                for j in range(NG)]

    g_wk = w_group(wa_hbm, wa, NG, 0)
    g_rest = (w_group(wa_hbm, wa, 2 * NG, 1) + w_group(wa_hbm, wa, 0, 1) + w_group(woa_hbm, woa, 0, 1)
              + w_group(wb_hbm, wb, 2 * NG, 1)
              + w_group(wb_hbm, wb, 0, 1) + w_group(wb_hbm, wb, NG, 1) + w_group(wob_hbm, wob, 0, 1))
    for c in g_wk:
        c.start()
    x_copy(0).start()
    x_copy(1).start()

    for i in range(8):
        zs[i] = 0
        zs[8 + i] = (i % 2) * KC

    def init_body(i, c):
        r0 = pl.multiple_of(i * 8, 8)
        for sb in sbufs:
            sb[pl.ds(r0, 8), :] = jnp.zeros((8, TQ), F32)
        g_acc[pl.ds(pl.multiple_of(i * 32, 32), 32), :] = jnp.zeros((32, D), F32)
        return c
    lax.fori_loop(0, 2 * KC // 8, init_body, 0)
    ot_buf[...] = jnp.zeros_like(ot_buf)
    l_buf[...] = jnp.ones_like(l_buf)
    m_ref[...] = jnp.zeros_like(m_ref)
    zp[...] = jnp.zeros_like(zp)
    acc_ref[...] = jnp.zeros_like(acc_ref)
    lc_ref[...] = jnp.zeros_like(lc_ref)

    def ln_tile(first, r0, dst, slot):
        rows = pl.ds(r0, HM)
        x = jnp.where(first, xb[rows, :].astype(F32), xres[rows, :])
        xres[rows, :] = x
        xn = _ln(x)
        for j in range(NG):
            dst[slot, j] = xn[:, j * 128:(j + 1) * 128]

    def ld_xn(src, slot):
        return jnp.concatenate([src[slot, j] for j in range(NG)], axis=1)

    def a_q(xn, p):
        return _phi(_dot(xn, _cat(wa, 2 * p, 2)))

    def a_k(xn):
        pk = _phi(_dot(xn, _cat(wa, NG, NG)))
        zrow = jnp.sum(pk.reshape(HM // 8, 8, D), axis=0)
        return pk.T.astype(BF16), zrow

    def a_mid():
        r = lax.broadcasted_iota(jnp.int32, (128, 128), 0) // DH
        c = lax.broadcasted_iota(jnp.int32, (128, 128), 1) // DH
        bd = r == c
        r16 = lax.broadcasted_iota(jnp.int32, (16, 128), 0)
        c16 = lax.broadcasted_iota(jnp.int32, (16, 128), 1) // DH
        kvs = []
        for g in range(NG):
            rows = slice(g * 128, (g + 1) * 128)
            kv = _dot(g_acc[rows, :].astype(BF16), wa[2 * NG + g])
            g_acc[rows, :] = jnp.zeros((128, D), F32)
            kvs.append(jnp.where(bd, kv, 0.0).astype(BF16))
            z = jnp.sum(zp[:, rows], axis=0, keepdims=True)
            zsel[g] = jnp.where(r16 == c16, jnp.broadcast_to(z, (16, 128)), 0.0).astype(BF16)
        zp[...] = jnp.zeros_like(zp)
        for g in range(NG):
            rows = slice(g * 128, (g + 1) * 128)
            mg = _dot(kvs[g], _cat(woa, 0, NG, rows)).astype(BF16)
            for j in range(NG):
                m_s[j, rows, :] = mg[:, j * 128:(j + 1) * 128]

    def a_norm(pq, g):
        den_t = _dot_nt(zsel[g], pq.astype(BF16))
        rd = _recip(den_t[0:8, :] + 1e-6)
        rb = jnp.concatenate([jnp.broadcast_to(rd[j:j + 1, :], (DH, HM)) for j in range(4)], axis=0)
        return (pq * rb.T).astype(BF16)

    def a_norm4(pqs, h):
        return [a_norm(pqs[g // 2][:, (g % 2) * 128:(g % 2 + 1) * 128], g) for g in range(4 * h, 4 * h + 4)]

    def a_out(pn, r0, p):
        rows = pl.ds(r0, HM)
        cols = slice(p * 256, (p + 1) * 256)
        x = xres[rows, cols] + _dot(pn, _cat(m_s, 2 * p, 2))
        xres[rows, cols] = x
        return x

    def b_proj(xn, r0, blk):
        rows = pl.ds(r0, HM)
        vt_s[blk] = pltpu.bitcast(_dot(xn, _cat(wb, 2 * NG, NG)).T.astype(BF16), jnp.uint32)
        qt = (_dot(xn, _cat(wb, 0, NG)) * QSCALE).T.astype(BF16)
        for g in range(NG):
            q_s[g, rows, :] = qt[g * 128:(g + 1) * 128, :]
        k = _dot(xn, _cat(wb, NG, NG)).astype(BF16)
        for g in range(NG):
            k_s[g, pl.ds(pl.multiple_of(blk * (HM // 2), HM // 2), HM // 2), :] = pltpu.bitcast(
                k[:, g * 128:(g + 1) * 128], jnp.uint32)

    def b_out(rows, c0, nb):
        cols = slice(c0 * 128, (c0 + nb) * 128)
        x = xres[rows, cols] + _dot(_cat(q_s, 0, NG, rows), _cat(wob, c0, nb))
        xres[rows, cols] = x
        xb[rows, cols] = x.astype(BF16)


    def tidx(t):
        gq = t // 4
        return gq // NQ, gq % NQ

    def get_q(t, j):
        g, qi = tidx(t)
        r0 = pl.multiple_of(qi * TQ, TQ)
        qh = jnp.concatenate([q_s[g, pl.ds(r0 + b * 128 + j * DH, DH), :] for b in range(TQ // 128)], axis=1)
        parts = []
        if j > 0:
            parts.append(jnp.zeros((j * DH, TQ), BF16))
        parts.append(qh)
        if j < 3:
            parts.append(jnp.zeros(((3 - j) * DH, TQ), BF16))
        return jnp.concatenate(parts, axis=0)

    def qk_chunk(t, qm, c, slot, m):
        g, _ = tidx(t)
        s = _dot(pltpu.bitcast(k_s[g, c * KC // 2:(c + 1) * KC // 2, :], BF16), qm)
        sbufs[c][pl.ds(slot, KC), :] = s
        cm = jnp.max(s.reshape(KC // 8, 8, TQ), axis=0)
        return cm if m is None else jnp.maximum(m, cm)

    def pv_chunk(t, j, c, slot, mb, acc, l):
        g, _ = tidx(t)
        s = sbufs[c][pl.ds(slot, KC), :]
        p = jnp.exp2(s.reshape(KC // 8, 8, TQ) - mb[None])
        a = l
        for r in range(7, -1, -1):
            pr = p[2 * r] + p[2 * r + 1]
            a = pr if a is None else a + pr
        pb = p.reshape(KC, TQ).astype(BF16)
        vt = pltpu.bitcast(vt_s[c, pl.ds(pl.multiple_of(g * 64 + j * (DH // 2), DH // 2), DH // 2), :], BF16)
        o = _dot(vt, pb)
        return (o if acc is None else acc + o), a

    def bcast_max(m):
        return jnp.broadcast_to(jnp.max(m, axis=0, keepdims=True), (8, TQ))

    def finalize(par, g, qi):
        parts = []
        for j in range(4):
            ls = jnp.sum(l_buf[par, j], axis=0, keepdims=True)
            parts.append(ot_buf[par, j * DH:(j + 1) * DH, :] * _recip(ls))
        ot = jnp.concatenate(parts, axis=0)
        q_s[g, pl.ds(pl.multiple_of(qi * TQ, TQ), TQ), :] = ot.T.astype(BF16)

    def slot_off(k):
        return pl.multiple_of(jnp.clip(zs[8 + (k & 7)], 0, KC), 8)

    def attention():
        def pv_finish(par, j, acc, l):
            ot_buf[par, j * DH:(j + 1) * DH, :] = acc
            l_buf[par, j] = l

        def body(i, carry):
            t0 = i * U
            mb_old = m_ref[0]
            mb = m_ref[1]
            acc = acc_ref[...]
            l = lc_ref[...]
            offs = [[slot_off(2 * i + 2 * a + b) for b in range(2)] for a in range(2)]
            for u in range(U):
                t = t0 + u
                ws = offs[0][u % 2]
                r1 = offs[1][(u + 1) % 2]
                r2 = offs[1][u % 2]
                tm1 = jnp.maximum(t - 1, 0)
                tm2 = jnp.maximum(t - 2, 0)
                qm = get_q(t, u % 4)
                m = None
                for c in range(NKC):
                    m = qk_chunk(t, qm, c, ws, m)
                    if c < LAG:
                        acc, l = pv_chunk(tm2, (u - 2) % 4, NKC - LAG + c, r2, mb_old, acc, l)
                        if c == LAG - 1:
                            pv_finish(((u - 2) // 4) % 2, (u - 2) % 4, acc, l)
                            acc = None
                            l = None
                    else:
                        acc, l = pv_chunk(tm1, (u - 1) % 4, c - LAG, r1, mb, acc, l)
                if u % 4 == 1:
                    g, qi = tidx(tm2)
                    if u == 1:
                        g = jnp.where(i == 0, NG, g)
                    finalize(((u - 2) // 4) % 2, g, qi)
                mb_old = mb
                mb = bcast_max(m)
            m_ref[0] = mb_old
            m_ref[1] = mb
            acc_ref[...] = acc
            lc_ref[...] = l
            return carry
        lax.fori_loop(0, NIT // U, body, 0)

        acc = acc_ref[...]
        l = lc_ref[...]
        todo = [(NIT - 2, 2, c, 0, 0) for c in range(NKC - LAG, NKC)] + [(NIT - 1, 3, c, KC, 1) for c in range(NKC)]
        npiece = 2 * NG
        lastp = 12
        n = 0
        for p in range(npiece):
            b_out(slice((p % 2) * (PO // 2), (p % 2 + 1) * (PO // 2)), p // 2, 1)
            upto = min(len(todo), -(-(p + 1) * len(todo) // (lastp + 1)))
            while n < upto:
                t, j, c, off, mi = todo[n]
                acc, l = pv_chunk(t, j, c, off, m_ref[mi], acc, l)
                if c == NKC - 1:
                    pv_finish(1, j, acc, l)
                    acc = None
                    l = None
                n += 1
            if p == lastp:
                finalize(1, NG - 1, NQ - 1)

    def pair(it, carry):
        first = it == 0

        @pl.when(first)
        def _():
            x_copy(0).wait()

        z0 = zs[1] & (NT_ROWS - 1)
        ln_tile(first, 0, xna, z0)
        ln_tile(first, HM, xnb, z0)

        @pl.when(first)
        def _():
            for c in g_wk:
                c.wait()
            for i in range(2, NT_ROWS):
                x_copy(i).start()

        def loop_a(i, c):
            @pl.when(jnp.logical_and(first, i + 1 < NT_ROWS))
            def _():
                x_copy(i + 1).wait()

            @pl.when(jnp.logical_and(first, i == 1))
            def _():
                for c in g_rest:
                    c.start()

            cur = (i + zs[i & 7]) & (NT_ROWS - 1)
            inx = jnp.minimum(i + 1, NT_ROWS - 1)
            nxt = (inx + zs[(i + 1) & 7]) & (NT_ROWS - 1)
            rn = pl.multiple_of(inx * TM, TM)
            pka, za = a_k(ld_xn(xna, cur))
            ln_tile(first, rn, xna, nxt)
            pkb, zb = a_k(ld_xn(xnb, cur))
            ln_tile(first, rn + HM, xnb, nxt)
            zp[...] += za + zb
            g_acc[...] += _dot(pka, ld_xn(xna, cur))
            g_acc[...] += _dot(pkb, ld_xn(xnb, cur))
            return c
        lax.fori_loop(0, NT_ROWS, loop_a, 0)

        @pl.when(first)
        def _():
            for c in g_rest:
                c.wait()

        a_mid()

        def loop2(i, c):
            ra = pl.multiple_of(i * TM, HM)
            rb = pl.multiple_of(i * TM + HM, HM)
            xa = ld_xn(xna, i)
            xb_ = ld_xn(xnb, i)
            pqa = [a_q(xa, p) for p in range(4)]
            pqb = [a_q(xb_, 0)]
            pna = a_norm4(pqa, 0)
            pqb.append(a_q(xb_, 1))
            pna += a_norm4(pqa, 1)
            pqb += [a_q(xb_, 2), a_q(xb_, 3)]
            pna = jnp.concatenate(pna, axis=1)
            ya = [a_out(pna, ra, 0)]
            pnb = a_norm4(pqb, 0)
            ya.append(a_out(pna, ra, 1))
            pnb += a_norm4(pqb, 1)
            ya += [a_out(pna, ra, 2), a_out(pna, ra, 3)]
            pnb = jnp.concatenate(pnb, axis=1)
            yb = [a_out(pnb, rb, p) for p in range(4)]
            b_proj(_ln(jnp.concatenate(ya, axis=1)), ra, 2 * i)
            b_proj(_ln(jnp.concatenate(yb, axis=1)), rb, 2 * i + 1)
            return c
        lax.fori_loop(0, NT_ROWS, loop2, 0)

        attention()

        @pl.when(it == 1)
        def _():
            out_copy(0, PO, 0).start()

        def loop_o(i, c):
            for hh in range(TO // HO):
                r0 = pl.multiple_of(PO + i * TO + hh * HO, 32)
                b_out(pl.ds(r0, HO), 0, NG)

                @pl.when(it == 1)
                def _():
                    out_copy(r0, HO, 1 + 2 * i + hh).start()
            return c
        lax.fori_loop(0, NO, loop_o, 0)
        return carry
    lax.fori_loop(0, 2, pair, 0)

    out_copy(0, PO, 0).wait()
    for i in range(2 * NO):
        out_copy(PO + i * HO, HO, i + 1).wait()


@jax.jit
def pallas_interleave_layers__linear_attn_block__mha_block__prompt_kernel(
    A_x: jax.Array,
    A_wqkv: jax.Array,
    A_wo: jax.Array,
    B_x: jax.Array,
    B_wqkv: jax.Array,
    B_wo: jax.Array,
):
    x = A_x.reshape(S, D)
    scratch = [
        pltpu.VMEM((S, D), BF16),
        pltpu.VMEM((S, D), F32),
        pltpu.VMEM((3 * NG, D, 128), BF16),
        pltpu.VMEM((NG, D, 128), BF16),
        pltpu.VMEM((3 * NG, D, 128), BF16),
        pltpu.VMEM((NG, D, 128), BF16),
        pltpu.VMEM((NG + 1, S, 128), BF16),
        pltpu.VMEM((NG, S // 2, 128), jnp.uint32),
        pltpu.VMEM((NKC, D // 2, 128), jnp.uint32),
        pltpu.VMEM((NT_ROWS, NG, HM, 128), BF16),
        pltpu.VMEM((NT_ROWS, NG, HM, 128), BF16),
        pltpu.VMEM((D, D), F32),
        pltpu.VMEM((8, D), F32),
        pltpu.VMEM((NG, D, 128), BF16),
        pltpu.VMEM((NG, 16, 128), BF16),
        pltpu.VMEM((2, 8, TQ), F32),
        pltpu.VMEM((DH, TQ), F32),
        pltpu.VMEM((8, TQ), F32),
        pltpu.VMEM((2, 128, TQ), F32),
        pltpu.VMEM((2, 4, 8, TQ), F32),
        pltpu.SMEM((16,), jnp.int32),
        pltpu.SemaphoreType.DMA((2 * NO + 1,)),
        pltpu.SemaphoreType.DMA((2,)),
    ] + [pltpu.VMEM((2 * KC, TQ), F32) for _ in range(NKC)]
    out = pl.pallas_call(
        _kernel,
        out_shape=jax.ShapeDtypeStruct((S, D), BF16),
        in_specs=[pl.BlockSpec(memory_space=pl.ANY)] * 5,
        out_specs=pl.BlockSpec(memory_space=pl.ANY),
        scratch_shapes=scratch,
        compiler_params=pltpu.CompilerParams(vmem_limit_bytes=110 * 1024 * 1024),
    )(x, A_wqkv, A_wo, B_wqkv, B_wo)
    return out.reshape(1, S, D)
```

```python
import math

import jax
import jax.numpy as jnp
from jax import lax
import jax.experimental.pallas as pl
import jax.experimental.pallas.tpu as pltpu

S, D, H, DH = 2048, 1024, 32, 32
NG = D // 128
TM = 256
HM = 128
NT_ROWS = S // TM
PO = 256
TO = 448
HO = 224
NO = (S - PO) // TO
TQ = 512
KC = 128
LAG = 3
U = 8
NQ = S // TQ
NKC = S // KC
NIT = H * NQ
QSCALE = (DH ** -0.5) * math.log2(math.e)
NT = (((1,), (1,)), ((), ()))
F32 = jnp.float32
BF16 = jnp.bfloat16


def _dot(a, b):
    return jnp.dot(a, b, preferred_element_type=F32)


def _dot_nt(a, b):
    return lax.dot_general(a, b, NT, preferred_element_type=F32)


def _phi(t):
    return jnp.where(t > 0, t + 1.0, jnp.exp(t)) + 1e-6


def _recip(d):
    return 1.0 / d


def _ln(x):
    m = jnp.mean(x, axis=-1, keepdims=True)
    xc = x - m
    v = jnp.mean(xc * xc, axis=-1, keepdims=True)
    return (xc * lax.rsqrt(v + 1e-5)).astype(BF16)


def _cat(ref, b0, n, rows=None):
    if rows is None:
        return jnp.concatenate([ref[b0 + j] for j in range(n)], axis=1)
    return jnp.concatenate([ref[b0 + j, rows, :] for j in range(n)], axis=1)


def _pack(x):
    return pltpu.bitcast(x, jnp.uint32)


def _unpack(x):
    return pltpu.bitcast(x, BF16)


def _kernel(x_hbm, wa_hbm, woa_hbm, wb_hbm, wob_hbm, out_hbm,
            xb, xres, wa, woa, wb, wob, q_s, k_s, vt_s,
            xna, xnb, g_acc, zp, m_s, zsel, m_ref, acc_ref, lc_ref, ot_buf, l_buf, zs, xsem, wsem, *sbufs):

    def x_copy(i):
        return pltpu.make_async_copy(x_hbm.at[pl.ds(i * TM, TM)], xb.at[pl.ds(i * TM, TM)], xsem.at[i])

    def out_copy(r0, n, k):
        return pltpu.make_async_copy(xb.at[pl.ds(r0, n)], out_hbm.at[pl.ds(r0, n)], xsem.at[k])

    def w_group(src, dst, b0, sem):
        return [pltpu.make_async_copy(src.at[:, pl.ds((b0 + j) * 128, 128)], dst.at[b0 + j], wsem.at[sem])
                for j in range(NG)]

    g_wk = w_group(wa_hbm, wa, NG, 0)
    g_rest = (w_group(wa_hbm, wa, 2 * NG, 1) + w_group(wa_hbm, wa, 0, 1) + w_group(woa_hbm, woa, 0, 1)
              + w_group(wb_hbm, wb, 2 * NG, 1)
              + w_group(wb_hbm, wb, 0, 1) + w_group(wb_hbm, wb, NG, 1) + w_group(wob_hbm, wob, 0, 1))
    for c in g_wk:
        c.start()
    x_copy(0).start()
    x_copy(1).start()

    for i in range(8):
        zs[i] = 0
        zs[8 + i] = (i % 2) * KC

    def init_body(i, c):
        r0 = pl.multiple_of(i * 8, 8)
        for sb in sbufs:
            sb[pl.ds(r0, 8), :] = jnp.zeros((8, TQ), F32)
        g_acc[pl.ds(pl.multiple_of(i * 32, 32), 32), :] = jnp.zeros((32, D), F32)
        xres[pl.ds(pl.multiple_of(i * 64, 64), 64), :] = jnp.zeros((64, D), F32)
        return c
    lax.fori_loop(0, 2 * KC // 8, init_body, 0)
    ot_buf[...] = jnp.zeros_like(ot_buf)
    l_buf[...] = jnp.ones_like(l_buf)
    m_ref[...] = jnp.zeros_like(m_ref)
    zp[...] = jnp.zeros_like(zp)
    acc_ref[...] = jnp.zeros_like(acc_ref)
    lc_ref[...] = jnp.zeros_like(lc_ref)

    def ln_tile(first, r0, dst, slot):
        rows = pl.ds(r0, HM)
        x = jnp.where(first, xb[rows, :].astype(F32), xres[rows, :])
        xres[rows, :] = x
        xn = _ln(x)
        for j in range(NG):
            dst[slot, j] = _pack(xn[:, j * 128:(j + 1) * 128])

    def ld_xn(src, slot):
        return jnp.concatenate([_unpack(src[slot, j]) for j in range(NG)], axis=1)

    def a_q(xn, p):
        return _phi(_dot(xn, _cat(wa, 2 * p, 2)))

    def a_k(xn):
        pk = _phi(_dot(xn, _cat(wa, NG, NG)))
        zrow = jnp.sum(pk.reshape(HM // 8, 8, D), axis=0)
        return pk.T.astype(BF16), zrow

    def a_mid():
        r = lax.broadcasted_iota(jnp.int32, (128, 128), 0) // DH
        c = lax.broadcasted_iota(jnp.int32, (128, 128), 1) // DH
        bd = r == c
        r16 = lax.broadcasted_iota(jnp.int32, (16, 128), 0)
        c16 = lax.broadcasted_iota(jnp.int32, (16, 128), 1) // DH
        kvs = []
        for g in range(NG):
            rows = slice(g * 128, (g + 1) * 128)
            kv = _dot(g_acc[rows, :].astype(BF16), wa[2 * NG + g])
            g_acc[rows, :] = jnp.zeros((128, D), F32)
            kvs.append(jnp.where(bd, kv, 0.0).astype(BF16))
            z = jnp.sum(zp[:, rows], axis=0, keepdims=True)
            zsel[g] = jnp.where(r16 == c16, jnp.broadcast_to(z, (16, 128)), 0.0).astype(BF16)
        zp[...] = jnp.zeros_like(zp)
        for g in range(NG):
            rows = slice(g * 128, (g + 1) * 128)
            mg = _dot(kvs[g], _cat(woa, 0, NG, rows)).astype(BF16)
            for j in range(NG):
                m_s[j, g * 64:(g + 1) * 64, :] = _pack(mg[:, j * 128:(j + 1) * 128])

    def a_norm(pq, g):
        den_t = _dot_nt(zsel[g], pq.astype(BF16))
        rd = _recip(den_t[0:8, :] + 1e-6)
        rb = jnp.concatenate([jnp.broadcast_to(rd[j:j + 1, :], (DH, HM)) for j in range(4)], axis=0)
        return (pq * rb.T).astype(BF16)

    def a_norm4(pqs, h):
        return [a_norm(pqs[g // 2][:, (g % 2) * 128:(g % 2 + 1) * 128], g) for g in range(4 * h, 4 * h + 4)]

    def a_out(pn, r0, p):
        rows = pl.ds(r0, HM)
        cols = slice(p * 256, (p + 1) * 256)
        x = xres[rows, cols] + _dot(pn, jnp.concatenate([_unpack(m_s[2 * p + j]) for j in range(2)], axis=1))
        xres[rows, cols] = x
        return x

    def b_proj(xn, r0, blk):
        vt_s[blk] = _pack(_dot(xn, _cat(wb, 2 * NG, NG)).T.astype(BF16))
        qt = (_dot(xn, _cat(wb, 0, NG)) * QSCALE).T.astype(BF16)
        for g in range(NG):
            q_s[g, pl.ds(pl.multiple_of(blk * (HM // 2), HM // 2), HM // 2), :] = _pack(qt[g * 128:(g + 1) * 128, :])
        k = _dot(xn, _cat(wb, NG, NG)).astype(BF16)
        for g in range(NG):
            k_s[g, pl.ds(pl.multiple_of(blk * (HM // 2), HM // 2), HM // 2), :] = pltpu.bitcast(
                k[:, g * 128:(g + 1) * 128], jnp.uint32)

    def b_out(h0, n, c0, nb):
        if isinstance(h0, int):
            rows = pl.ds(2 * h0, n)
        else:
            rows = pl.ds(pl.multiple_of(2 * h0, 32), n)
        cols = slice(c0 * 128, (c0 + nb) * 128)
        o = jnp.concatenate([_unpack(q_s[g, pl.ds(h0, n // 2), :]) for g in range(NG)], axis=1)
        x = xres[rows, cols] + _dot(o, _cat(wob, c0, nb))
        xres[rows, cols] = x
        xb[rows, cols] = x.astype(BF16)


    def tidx(t):
        return t >> 4, (t >> 2) & (NQ - 1)

    def get_q(t, j):
        g, qi = tidx(t)
        r0 = pl.multiple_of(qi * (TQ // 2), TQ // 2)
        qh = jnp.concatenate([_unpack(q_s[g, pl.ds(r0 + b * 64 + j * (DH // 2), DH // 2), :])
                              for b in range(TQ // 128)], axis=1)
        parts = []
        if j > 0:
            parts.append(jnp.zeros((j * DH, TQ), BF16))
        parts.append(qh)
        if j < 3:
            parts.append(jnp.zeros(((3 - j) * DH, TQ), BF16))
        return jnp.concatenate(parts, axis=0)

    def qk_chunk(t, qm, c, slot, m):
        g, _ = tidx(t)
        s = _dot(pltpu.bitcast(k_s[g, c * KC // 2:(c + 1) * KC // 2, :], BF16), qm)
        sbufs[c][pl.ds(slot, KC), :] = s
        s3 = s.reshape(KC // 8, 8, TQ)
        for r in range(KC // 8):
            m = s3[r] if m is None else jnp.maximum(m, s3[r])
        return m

    def pv_chunk(t, j, c, slot, mb, acc, l):
        g, _ = tidx(t)
        s = sbufs[c][pl.ds(slot, KC), :]
        p = jnp.exp2(s.reshape(KC // 8, 8, TQ) - mb[None])
        a = l
        for r in range(7, -1, -1):
            pr = p[2 * r] + p[2 * r + 1]
            a = pr if a is None else a + pr
        pb = p.reshape(KC, TQ).astype(BF16)
        vt = pltpu.bitcast(vt_s[c, pl.ds(pl.multiple_of(g * 64 + j * (DH // 2), DH // 2), DH // 2), :], BF16)
        o = _dot(vt, pb)
        return (o if acc is None else acc + o), a

    def bcast_max(m):
        return jnp.broadcast_to(jnp.max(m, axis=0, keepdims=True), (8, TQ))

    def finalize(par, g, qi):
        parts = []
        for j in range(4):
            ls = jnp.sum(l_buf[par, j], axis=0, keepdims=True)
            parts.append(ot_buf[par, j * DH:(j + 1) * DH, :] * _recip(ls))
        ot = jnp.concatenate(parts, axis=0)
        q_s[g, pl.ds(pl.multiple_of(qi * (TQ // 2), TQ // 2), TQ // 2), :] = _pack(ot.T.astype(BF16))

    def slot_off(k):
        return pl.multiple_of(jnp.clip(zs[8 + (k & 7)], 0, KC), 8)

    def attention():
        def pv_finish(par, j, acc, l):
            ot_buf[par, j * DH:(j + 1) * DH, :] = acc
            l_buf[par, j] = l

        def body(i, carry):
            t0 = i * U
            mb_old = m_ref[0]
            mb = m_ref[1]
            acc = acc_ref[...]
            l = lc_ref[...]
            offs = [[slot_off(2 * i + 2 * a + b) for b in range(2)] for a in range(2)]
            for u in range(U):
                t = t0 + u
                ws = offs[0][u % 2]
                r1 = offs[1][(u + 1) % 2]
                r2 = offs[1][u % 2]
                tm1 = jnp.maximum(t - 1, 0)
                tm2 = jnp.maximum(t - 2, 0)
                qm = get_q(t, u % 4)
                m = None
                for c in range(NKC):
                    m = qk_chunk(t, qm, c, ws, m)
                    if c < LAG:
                        acc, l = pv_chunk(tm2, (u - 2) % 4, NKC - LAG + c, r2, mb_old, acc, l)
                        if c == LAG - 1:
                            pv_finish(((u - 2) // 4) % 2, (u - 2) % 4, acc, l)
                            acc = None
                            l = None
                    else:
                        acc, l = pv_chunk(tm1, (u - 1) % 4, c - LAG, r1, mb, acc, l)
                if u % 4 == 1:
                    g, qi = tidx(tm2)
                    if u == 1:
                        g = jnp.where(i == 0, NG, g)
                    finalize(((u - 2) // 4) % 2, g, qi)
                mb_old = mb
                mb = bcast_max(m)
            m_ref[0] = mb_old
            m_ref[1] = mb
            acc_ref[...] = acc
            lc_ref[...] = l
            return carry
        lax.fori_loop(0, NIT // U, body, 0)

        acc = acc_ref[...]
        l = lc_ref[...]
        todo = [(NIT - 2, 2, c, 0, 0) for c in range(NKC - LAG, NKC)] + [(NIT - 1, 3, c, KC, 1) for c in range(NKC)]
        npiece = 2 * NG
        lastp = 12
        n = 0
        for p in range(npiece):
            b_out((p % 2) * (PO // 4), PO // 2, p // 2, 1)
            upto = min(len(todo), -(-(p + 1) * len(todo) // (lastp + 1)))
            while n < upto:
                t, j, c, off, mi = todo[n]
                acc, l = pv_chunk(t, j, c, off, m_ref[mi], acc, l)
                if c == NKC - 1:
                    pv_finish(1, j, acc, l)
                    acc = None
                    l = None
                n += 1
            if p == lastp:
                finalize(1, NG - 1, NQ - 1)

    def pair(it, carry):
        first = it == 0

        @pl.when(first)
        def _():
            x_copy(0).wait()

        z0 = zs[1] & (NT_ROWS - 1)
        ln_tile(first, 0, xna, z0)
        ln_tile(first, HM, xnb, z0)

        @pl.when(first)
        def _():
            for c in g_wk:
                c.wait()
            for i in range(2, NT_ROWS):
                x_copy(i).start()

        def loop_a(i, c):
            inx = jnp.minimum(i + 1, NT_ROWS - 1)

            @pl.when(jnp.logical_and(first, i + 1 < NT_ROWS))
            def _():
                x_copy(inx).wait()

            @pl.when(jnp.logical_and(first, i == 1))
            def _():
                for c in g_rest:
                    c.start()

            cur = (i + zs[i & 7]) & (NT_ROWS - 1)
            nxt = (inx + zs[(i + 1) & 7]) & (NT_ROWS - 1)
            rn = pl.multiple_of(inx * TM, TM)
            pka, za = a_k(ld_xn(xna, cur))
            ln_tile(first, rn, xna, nxt)
            pkb, zb = a_k(ld_xn(xnb, cur))
            ln_tile(first, rn + HM, xnb, nxt)
            zp[...] += za + zb
            g_acc[...] += _dot(pka, ld_xn(xna, cur))
            g_acc[...] += _dot(pkb, ld_xn(xnb, cur))
            return c
        lax.fori_loop(0, NT_ROWS, loop_a, 0)

        @pl.when(first)
        def _():
            for c in g_rest:
                c.wait()

        a_mid()

        def loop2(i, c):
            ra = pl.multiple_of(i * TM, HM)
            rb = pl.multiple_of(i * TM + HM, HM)
            xa = ld_xn(xna, i)
            xb_ = ld_xn(xnb, i)
            pqa = [a_q(xa, p) for p in range(4)]
            pqb = [a_q(xb_, 0)]
            pna = a_norm4(pqa, 0)
            pqb.append(a_q(xb_, 1))
            pna += a_norm4(pqa, 1)
            pqb += [a_q(xb_, 2), a_q(xb_, 3)]
            pna = jnp.concatenate(pna, axis=1)
            ya = [a_out(pna, ra, 0)]
            pnb = a_norm4(pqb, 0)
            ya.append(a_out(pna, ra, 1))
            pnb += a_norm4(pqb, 1)
            ya += [a_out(pna, ra, 2), a_out(pna, ra, 3)]
            pnb = jnp.concatenate(pnb, axis=1)
            yb = [a_out(pnb, rb, p) for p in range(4)]
            b_proj(_ln(jnp.concatenate(ya, axis=1)), ra, 2 * i)
            b_proj(_ln(jnp.concatenate(yb, axis=1)), rb, 2 * i + 1)
            return c
        lax.fori_loop(0, NT_ROWS, loop2, 0)

        attention()

        @pl.when(it == 1)
        def _():
            out_copy(0, PO, 0).start()

        def loop_o(i, c):
            for hh in range(TO // HO):
                r0 = pl.multiple_of(PO + i * TO + hh * HO, 32)
                b_out(pl.multiple_of((PO + hh * HO) // 2 + i * (TO // 2), 16), HO, 0, NG)

                @pl.when(it == 1)
                def _():
                    out_copy(r0, HO, 1 + 2 * i + hh).start()
            return c
        lax.fori_loop(0, NO, loop_o, 0)
        return carry
    lax.fori_loop(0, 2, pair, 0)

    out_copy(0, PO, 0).wait()
    for i in range(2 * NO):
        out_copy(PO + i * HO, HO, i + 1).wait()


@jax.jit
def pallas_interleave_layers__linear_attn_block__mha_block__prompt_kernel(
    A_x: jax.Array,
    A_wqkv: jax.Array,
    A_wo: jax.Array,
    B_x: jax.Array,
    B_wqkv: jax.Array,
    B_wo: jax.Array,
):
    x = A_x.reshape(S, D)
    scratch = [
        pltpu.VMEM((S, D), BF16),
        pltpu.VMEM((S, D), F32),
        pltpu.VMEM((3 * NG, D, 128), BF16),
        pltpu.VMEM((NG, D, 128), BF16),
        pltpu.VMEM((3 * NG, D, 128), BF16),
        pltpu.VMEM((NG, D, 128), BF16),
        pltpu.VMEM((NG + 1, S // 2, 128), jnp.uint32),
        pltpu.VMEM((NG, S // 2, 128), jnp.uint32),
        pltpu.VMEM((NKC, D // 2, 128), jnp.uint32),
        pltpu.VMEM((NT_ROWS, NG, HM // 2, 128), jnp.uint32),
        pltpu.VMEM((NT_ROWS, NG, HM // 2, 128), jnp.uint32),
        pltpu.VMEM((D, D), F32),
        pltpu.VMEM((8, D), F32),
        pltpu.VMEM((NG, D // 2, 128), jnp.uint32),
        pltpu.VMEM((NG, 16, 128), BF16),
        pltpu.VMEM((2, 8, TQ), F32),
        pltpu.VMEM((DH, TQ), F32),
        pltpu.VMEM((8, TQ), F32),
        pltpu.VMEM((2, 128, TQ), F32),
        pltpu.VMEM((2, 4, 8, TQ), F32),
        pltpu.SMEM((16,), jnp.int32),
        pltpu.SemaphoreType.DMA((2 * NO + 1,)),
        pltpu.SemaphoreType.DMA((2,)),
    ] + [pltpu.VMEM((2 * KC, TQ), F32) for _ in range(NKC)]
    out = pl.pallas_call(
        _kernel,
        out_shape=jax.ShapeDtypeStruct((S, D), BF16),
        in_specs=[pl.BlockSpec(memory_space=pl.ANY)] * 5,
        out_specs=pl.BlockSpec(memory_space=pl.ANY),
        scratch_shapes=scratch,
        compiler_params=pltpu.CompilerParams(vmem_limit_bytes=110 * 1024 * 1024),
    )(x, A_wqkv, A_wo, B_wqkv, B_wo)
    return out.reshape(1, S, D)
```
